```python
import jax
import jax.numpy as jnp

def _softmax(x, axis=-1):
    return jax.nn.softmax(x, axis=axis)
def _gelu(x):
    return jax.nn.gelu(x, approximate=True)
def _silu(x):
    return jax.nn.silu(x)
def _sigmoid(x):
    return jax.nn.sigmoid(x)
def _layernorm(x, axis=-1, eps=1e-5):
    m = jnp.mean(x, axis=axis, keepdims=True)
    v = jnp.var(x, axis=axis, keepdims=True)
    return (x - m) / jnp.sqrt(v + eps)
def _scatter_add(tgt, idx, src, axis=0):
    return tgt.at[idx].add(src)
def _segment_sum(src, seg, n):
    return jax.ops.segment_sum(src, seg, n)
class _Rng:
    def __init__(self, key):
        self._k = key
    def _next(self):
        self._k, sub = jax.random.split(self._k)
        return sub
    def normal(self, shape):
        return jax.random.normal(self._next(), shape, dtype=jnp.bfloat16)
    def randint(self, lo, hi, shape):
        return jax.random.randint(self._next(), shape, lo, hi, dtype=jnp.int32)
    def uniform(self, shape, lo=0.0, hi=1.0):
        return jax.random.uniform(self._next(), shape, jnp.bfloat16, lo, hi)
    def permutation(self, n):
        return jax.random.permutation(self._next(), n)


kernel_name = 'standalone__batchnorm__sampling'

def setup_inputs():
    _rng = _Rng(jax.random.key(int.from_bytes(__import__("os").urandom(4), "little")))
    _w = (lambda a: (lambda t: t.astype(jnp.bfloat16) if jnp.issubdtype(t.dtype, jnp.floating) else t)(jnp.asarray(a)))
    B, S, C = 1024, 32, 576
    K = 3
    return {
        "x": _w((lambda *s: _rng.normal(s) * 0.05)(B, S, C)),
        "w": _w((lambda *s: _rng.normal(s) * 0.05)(K, C, C) * (1.0 / (K * C) ** 0.5)),
        "mean": _w((lambda *s: _rng.normal(s) * 0.05)(C) * 0.1),
        "var": _w(jnp.abs((lambda *s: _rng.normal(s) * 0.05)(C)) + 0.5),
        "g": _w((lambda *s: _rng.normal(s) * 0.05)(C) + 1.0),
        "b": _w((lambda *s: _rng.normal(s) * 0.05)(C) * 0.1),
    }

def reference(x, w, mean, var, g, b):
    K = 3
    P = K // 2
    S = x.shape[1]
    xp = jnp.pad(x, ((0, 0), (P, P), (0, 0)))
    y = sum(jnp.einsum('bsc,cd->bsd', xp[:, k:k + S, :], w[k]) for k in range(K))
    inv_std = 1.0 / jnp.sqrt(var + 1e-5)
    y = (y - mean) * (g * inv_std) + b
    return _silu(y)
```

```python
import jax
import jax.numpy as jnp
import jax.experimental.pallas as pl
import jax.experimental.pallas.tpu as pltpu


@jax.jit
def pallas_standalone__batchnorm__sampling_kernel(
    x: jax.Array,
    w: jax.Array,
    mean: jax.Array,
    var: jax.Array,
    g: jax.Array,
    b: jax.Array,
):
    B, S, C = x.shape
    K = w.shape[0]
    bn = 128

    def kernel(x_ref, w_ref, mean_ref, var_ref, g_ref, b_ref, o_ref,
               wt_ref, wt12_ref, sc_ref, sh_ref):
        @pl.when(pl.program_id(0) == 0)
        def _():
            wf = w_ref[...].reshape(K * C, C)
            wt_ref[...] = wf.T
            wt12_ref[...] = wf[C:, :].T
            sc = g_ref[...].astype(jnp.float32) / jnp.sqrt(var_ref[...].astype(jnp.float32) + 1e-5)
            sh = b_ref[...].astype(jnp.float32) - mean_ref[...].astype(jnp.float32) * sc
            sc_ref[...] = jnp.broadcast_to(sc, (bn, C)).T
            sh_ref[...] = jnp.broadcast_to(sh, (bn, C)).T

        def epilogue(y, s):
            y = y * sc_ref[...] + sh_ref[...]
            o_ref[s] = (y * jax.nn.sigmoid(y)).astype(o_ref.dtype)

        def mm(a, c):
            return jnp.dot(a, c, preferred_element_type=jnp.float32)

        epilogue(mm(wt12_ref[...], x_ref[pl.ds(0, 2)].reshape(2 * C, bn)), 0)
        for s in range(1, S - 1):
            epilogue(mm(wt_ref[...], x_ref[pl.ds(s - 1, 3)].reshape(K * C, bn)), s)
        epilogue(mm(wt_ref[:, pl.ds(0, 2 * C)], x_ref[pl.ds(S - 2, 2)].reshape(2 * C, bn)), S - 1)

    vec = pl.BlockSpec((1, C), lambda i: (0, 0))
    out = pl.pallas_call(
        kernel,
        grid=(B // bn,),
        in_specs=[pl.BlockSpec((S, C, bn), lambda i: (0, 0, i)),
                  pl.BlockSpec((K, C, C), lambda i: (0, 0, 0)), vec, vec, vec, vec],
        out_specs=pl.BlockSpec((S, C, bn), lambda i: (0, 0, i)),
        out_shape=jax.ShapeDtypeStruct((S, C, B), x.dtype),
        scratch_shapes=[pltpu.VMEM((C, K * C), w.dtype), pltpu.VMEM((C, 2 * C), w.dtype),
                        pltpu.VMEM((C, bn), jnp.float32), pltpu.VMEM((C, bn), jnp.float32)],
        compiler_params=pltpu.CompilerParams(
            dimension_semantics=("arbitrary",), vmem_limit_bytes=100 * 2**20),
    )(jnp.transpose(x, (1, 2, 0)), w, mean.reshape(1, C), var.reshape(1, C),
      g.reshape(1, C), b.reshape(1, C))
    return jnp.transpose(out, (2, 0, 1))
```

```python
import jax
import jax.numpy as jnp
import jax.experimental.pallas as pl
import jax.experimental.pallas.tpu as pltpu


_A = 2.0 / 3.0
_BN = 128
_SPLIT = 13


@jax.jit
def pallas_standalone__batchnorm__sampling_kernel(
    x: jax.Array,
    w: jax.Array,
    mean: jax.Array,
    var: jax.Array,
    g: jax.Array,
    b: jax.Array,
):
    B, S, C = x.shape
    K = w.shape[0]
    f32, bf16, u32 = jnp.float32, jnp.bfloat16, jnp.uint32
    bn = _BN
    NT, NQ = B // bn, S // 4
    a_, b_ = _A, 1.0 / _A
    a2, b2 = a_ * a_, b_ * b_
    s2 = a2 + b2
    Na, Nb = 2 * a2 * (a2 - b2), 2 * b2 * (b2 - a2)
    r = b_ / a_

    def kernel(x_hbm, w_hbm, mean_hbm, var_hbm, g_hbm, b_hbm, o_hbm,
               xb, ob, wb, v0, v1, v2, v3, gt_ref, sc_ref, sh_ref, xsem, osem, wsem):
        def lanes(i):
            if isinstance(i, int):
                return pl.ds(i * bn, bn)
            return pl.ds(pl.multiple_of(i * bn, bn), bn)

        def x_copy(i, slot, p):
            lo, n = ((0, _SPLIT), (_SPLIT, S - _SPLIT))[p]
            return pltpu.make_async_copy(
                x_hbm.at[pl.ds(lo, n), :, lanes(i)], xb.at[slot, pl.ds(lo, n)], xsem.at[slot, p])

        def o_copy(i, slot, lo, n):
            return pltpu.make_async_copy(
                ob.at[slot, pl.ds(lo, n)], o_hbm.at[pl.ds(lo, n), :, lanes(i)], osem.at[slot])

        def o_wait_all(slot):
            pltpu.make_async_copy(ob.at[slot], ob.at[slot], osem.at[slot]).wait()

        def group(slot, q):
            def ld(j):
                return xb[slot, 4 * q - 1 + j].astype(f32)
            d1, d2, d3, d4 = ld(1), ld(2), ld(3), ld(4)
            D0 = d4 - s2 * d2
            if q > 0:
                D0 = D0 + ld(0)
            D5 = d1 - s2 * d3
            if q < NQ - 1:
                D5 = D5 + ld(5)
            D5 = D5 * (1 / a_ ** 3)
            ea, eb = d4 - a2 * d2, d4 - b2 * d2
            u, v = a_ * d3 - b_ * d1, b_ * d3 - a_ * d1
            Ds = [t.astype(bf16) for t in (D0, eb + u, eb - u, ea + v, ea - v, D5)]
            m = [None] * 6
            for p in (0, 5, 1, 2, 3, 4):
                m[p] = jnp.dot(pltpu.bitcast(gt_ref[p], bf16), Ds[p], preferred_element_type=f32)

            def epilogue(y, j):
                h = y * sc_ref[j] + sh_ref[...]
                ob[slot, 4 * q + j] = (h * jnp.tanh(h) + h).astype(ob.dtype)
            Pa, Qa, Pb, Qb = m[1] + m[2], m[1] - m[2], m[3] + m[4], m[3] - m[4]
            epilogue(m[0] + Pa + Pb, 0)
            epilogue(Qa + r * Qb, 1)
            epilogue(Pa + (r * r) * Pb, 2)
            epilogue(Qa + (r ** 3) * Qb + m[5], 3)

        vb = (v0, v1, v2, v3)
        vc = [pltpu.make_async_copy(h, vb[k], wsem.at[k])
              for k, h in enumerate((mean_hbm, var_hbm, g_hbm, b_hbm))]
        wc = [pltpu.make_async_copy(w_hbm.at[k], wb.at[k], wsem.at[4 + k]) for k in range(K)]
        for k in (0, 2, 1):
            wc[k].start()
        for c in vc:
            c.start()
        x_copy(0, 0, 0).start()
        for c in vc:
            c.wait()
        mean_v, var_v, g_v, b_v = (vb[k][...].astype(f32).reshape(1, C) for k in range(4))
        sc = g_v / jnp.sqrt(var_v + 1e-5)
        sh = b_v - mean_v * sc
        scb = jnp.broadcast_to(sc, (bn, C)).T
        for j in range(4):
            sc_ref[j] = scb * (0.5 * a_ ** j)
        sh_ref[...] = 0.5 * jnp.broadcast_to(sh, (bn, C)).T
        wc[0].wait()
        x_copy(0, 0, 1).start()
        wt0 = wb[0].T
        gt_ref[0] = pltpu.bitcast(wt0, u32)
        wc[2].wait()
        wt2 = wb[2].T
        gt_ref[5] = pltpu.bitcast(wt2, u32)
        g0, g2 = wt0.astype(f32), wt2.astype(f32)
        ea, eb = g0 * (1 / Na) + g2 * (a2 / Na), g0 * (1 / Nb) + g2 * (b2 / Nb)
        wc[1].wait()
        g1 = wb[1].T.astype(f32)
        oa, ob_ = g1 * (a_ / Na), g1 * (b_ / Nb)
        for p, t in ((1, ea + oa), (2, ea - oa), (3, eb + ob_), (4, eb - ob_)):
            gt_ref[p] = pltpu.bitcast(t.astype(bf16), u32)

        def tile(i, carry):
            slot = i % 2

            @pl.when(i + 1 < NT)
            def _():
                x_copy(i + 1, 1 - slot, 0).start()
                x_copy(i + 1, 1 - slot, 1).start()

            @pl.when(i >= 2)
            def _():
                o_wait_all(slot)
            x_copy(i, slot, 0).wait()
            done = 0
            for q in range(NQ):
                if q == 2:
                    x_copy(i, slot, 1).wait()
                group(slot, q)
                if q >= 3:
                    o_copy(i, slot, done, 4 * (q + 1) - done).start()
                    done = 4 * (q + 1)
            return carry

        jax.lax.fori_loop(0, NT, tile, 0)
        o_wait_all(0)
        o_wait_all(1)

    hbm = pl.BlockSpec(memory_space=pltpu.HBM)
    out = pl.pallas_call(
        kernel,
        in_specs=[hbm] * 6,
        out_specs=hbm,
        out_shape=jax.ShapeDtypeStruct((S, C, B), x.dtype),
        scratch_shapes=[
            pltpu.VMEM((2, S, C, bn), x.dtype),
            pltpu.VMEM((2, S, C, bn), x.dtype),
            pltpu.VMEM((K, C, C), w.dtype),
            *[pltpu.VMEM((C,), mean.dtype)] * 4,
            pltpu.VMEM((6, C // 2, C), u32),
            pltpu.VMEM((4, C, bn), f32),
            pltpu.VMEM((C, bn), f32),
            pltpu.SemaphoreType.DMA((2, 2)),
            pltpu.SemaphoreType.DMA((2,)),
            pltpu.SemaphoreType.DMA((4 + K,)),
        ],
        compiler_params=pltpu.CompilerParams(vmem_limit_bytes=64 * 2**20),
    )(jnp.transpose(x, (1, 2, 0)), w, mean, var, g, b)
    return jnp.transpose(out, (2, 0, 1))
```
